```python
import jax
import jax.numpy as jnp

def _softmax(x, axis=-1):
    return jax.nn.softmax(x, axis=axis)
def _gelu(x):
    return jax.nn.gelu(x, approximate=True)
def _silu(x):
    return jax.nn.silu(x)
def _sigmoid(x):
    return jax.nn.sigmoid(x)
def _layernorm(x, axis=-1, eps=1e-5):
    m = jnp.mean(x, axis=axis, keepdims=True)
    v = jnp.var(x, axis=axis, keepdims=True)
    return (x - m) / jnp.sqrt(v + eps)
def _scatter_add(tgt, idx, src, axis=0):
    return tgt.at[idx].add(src)
def _segment_sum(src, seg, n):
    return jax.ops.segment_sum(src, seg, n)
class _Rng:
    def __init__(self, key):
        self._k = key
    def _next(self):
        self._k, sub = jax.random.split(self._k)
        return sub
    def normal(self, shape):
        return jax.random.normal(self._next(), shape, dtype=jnp.bfloat16)
    def randint(self, lo, hi, shape):
        return jax.random.randint(self._next(), shape, lo, hi, dtype=jnp.int32)
    def uniform(self, shape, lo=0.0, hi=1.0):
        return jax.random.uniform(self._next(), shape, jnp.bfloat16, lo, hi)
    def permutation(self, n):
        return jax.random.permutation(self._next(), n)


kernel_name = 'standalone__qk_norm__prompt'

def setup_inputs():
    _rng = _Rng(jax.random.key(int.from_bytes(__import__("os").urandom(4), "little")))
    _w = (lambda a: (lambda t: t.astype(jnp.bfloat16) if jnp.issubdtype(t.dtype, jnp.floating) else t)(jnp.asarray(a)))
    B, H, S, D = 2, 32, 2048, 1024
    Dh = D // H
    return {
        "q": _w((lambda *s: _rng.normal(s) * 0.05)(B, H, S, Dh)),
        "k": _w((lambda *s: _rng.normal(s) * 0.05)(B, H, S, Dh)),
        "v": _w((lambda *s: _rng.normal(s) * 0.05)(B, H, S, Dh)),
        "t": _w(jnp.abs((lambda *s: _rng.normal(s) * 0.05)(H)) + 1.0),
    }

def reference(q, k, v, t):
    eps = 1e-6
    qn = q / (jnp.sqrt((q * q).sum(axis=-1, keepdims=True)) + eps)
    kn = k / (jnp.sqrt((k * k).sum(axis=-1, keepdims=True)) + eps)
    logits = jnp.einsum('bhqd,bhkd->bhqk', qn, kn) * t[None, :, None, None]
    attn = _softmax(logits, axis=-1)
    return jnp.einsum('bhqk,bhkd->bhqd', attn, v)
```

```python
import functools

import jax
import jax.numpy as jnp
import numpy as np
from jax import lax
from jax.experimental import pallas as pl
from jax.experimental.pallas import tpu as pltpu

f32 = jnp.float32
bf16 = jnp.bfloat16
u32 = jnp.uint32

EPS = 1e-6
LOG2E = 1.4426950408889634
T_SAFE = 16.0

CH = 128
BQ = 512


def make_kernel(B, H, S, D, BK=256, LAG=2, HB=4, NPRE=4, KLEAD=4, OUT_ITERS=(1, 8, 14)):
    BH = B * H
    NC = S // CH
    NP = S // BQ
    NBLK = S // BK
    assert D == 32 and S % BQ == 0 and S % BK == 0 and BK % CH == 0
    assert (BH - NPRE) % HB == 0
    assert (KLEAD - 1) * CH // BK <= NBLK - 2 - LAG
    assert LAG + (KLEAD * CH + BK - 1) // BK + 1 <= NBLK

    def kernel(t_ref, q_hbm, k_hbm, v_hbm, o_hbm,
               q_v, k_v, v_v, o_v, kn, qn, vn, in_sem, out_sem):

        def in_copies(lo, n, si):
            return [pltpu.make_async_copy(src.at[pl.ds(lo, n)], dst.at[pl.ds(lo, n)], in_sem.at[si])
                    for src, dst in ((k_hbm, k_v), (q_hbm, q_v), (v_hbm, v_v))]

        def start_in(lo, n, si):
            for cp in in_copies(lo, n, si):
                cp.start()

        def wait_in(lo, n, si):
            for cp in in_copies(lo, n, si):
                cp.wait()

        def out_copy(lo, n):
            return pltpu.make_async_copy(o_v.at[pl.ds(lo, n)], o_hbm.at[pl.ds(lo, n)], out_sem.at[0])

        def normalise(x_bf16, scale):
            x = x_bf16.astype(f32)
            ss = jnp.sum(x * x, axis=0, keepdims=True)
            return x * (scale / (jnp.sqrt(ss) + EPS))

        def prep_kv(h, c):
            cols = slice(c * CH, (c + 1) * CH)
            kk = normalise(k_v[h, :, cols], 1.0)
            row = lax.broadcasted_iota(jnp.int32, (8, CH), 0)
            one = jnp.where(row == 0, 1.0, 0.0).astype(f32)
            y = jnp.concatenate([kk, one, jnp.zeros((128 - D - 8, CH), f32)], axis=0)
            kn[c * (CH // 2):(c + 1) * (CH // 2), :] = pltpu.bitcast(y.T.astype(bf16), u32)
            vn[:, cols] = pltpu.bitcast(v_v[h, :, cols], u32)

        def prep_q(h, j):
            cols = slice(j * BQ, (j + 1) * BQ)
            c = t_ref[h % H] * LOG2E
            qq = normalise(q_v[h, :, cols], c)
            qn[0:D // 2, cols] = pltpu.bitcast(qq.astype(bf16), u32)
            row = lax.broadcasted_iota(jnp.int32, (16, BQ), 0)
            sh = jnp.where(row == 0, -jnp.abs(c), 0.0).astype(f32)
            qn[D // 2:D // 2 + 8, cols] = pltpu.bitcast(sh.astype(bf16), u32)

        def qk_exp(j, kb):
            w = jnp.concatenate([qn[:, j * BQ:(j + 1) * BQ], jnp.zeros((64 - D // 2 - 8, BQ), u32)], axis=0)
            kk = pltpu.bitcast(kn[kb * (BK // 2):(kb + 1) * (BK // 2), :], bf16)
            s = jnp.dot(kk, pltpu.bitcast(w, bf16), preferred_element_type=f32)
            p = jnp.exp2(s)
            return jnp.sum(p.reshape(BK // 8, 8, BQ), axis=0), p.astype(bf16)

        def pv(kb, p):
            vv = pltpu.bitcast(vn[:, kb * BK:(kb + 1) * BK], bf16)
            return jnp.dot(vv, p, preferred_element_type=f32)

        def finish(h, j, l, acc):
            lt = jnp.sum(l, axis=0, keepdims=True)
            o_v[h, :, j * BQ:(j + 1) * BQ] = (acc * (1.0 / lt)).astype(bf16)

        def run_heads(heads):
            blocks = []
            for h in heads:
                hn = jnp.minimum(h + 1, BH - 1)
                for j in range(NP):
                    pre = [[] for _ in range(NBLK)]
                    if j == 0:
                        for c in range(KLEAD, NC):
                            pre[(c - KLEAD) * CH // BK].append(functools.partial(prep_kv, h, c))
                    if j + 1 < NP:
                        pre[NBLK // 2].append(functools.partial(prep_q, h, j + 1))
                    else:
                        pre[NBLK // 2].append(functools.partial(prep_q, hn, 0))
                        for c in range(KLEAD):
                            pre[NBLK - 1].append(functools.partial(prep_kv, hn, c))
                    for kb in range(NBLK):
                        blocks.append((h, j, kb, pre[kb]))
            pend = {}
            l = l_done = acc = None
            for i in range(len(blocks) + LAG):
                if i < len(blocks):
                    h, j, kb, pre = blocks[i]
                    for f in pre:
                        f()
                    ps, pend[i] = qk_exp(j, kb)
                    l = ps if kb == 0 else l + ps
                    if kb == NBLK - 1:
                        l_done = l
                if i >= LAG:
                    h, j, kb, _ = blocks[i - LAG]
                    r = pv(kb, pend.pop(i - LAG))
                    acc = r if kb == 0 else acc + r
                    if kb == NBLK - 1:
                        finish(h, j, l_done, acc)
            assert LAG < NBLK

        def fast_path():
            for c in range(KLEAD):
                prep_kv(0, c)
            prep_q(0, 0)
            wait_in(1, 1, 1)
            na = NPRE + HB + 1
            start_in(2, na - 2, 0)
            nwide = (BH - NPRE) // HB
            segs = [((0, 1), (0, 0))]
            cuts = [1] + [x for x in OUT_ITERS if x > 1] + [nwide]
            segs.append(((1, NPRE), (0, 1)))
            for a, b in zip(cuts[:-1], cuts[1:]):
                segs.append(((0, 0), (a, b)))
            acts = [[] for _ in segs]
            acts[1] += [functools.partial(wait_in, 2, na - 2, 0), functools.partial(start_in, na, BH - na, 1)]
            acts[2] += [functools.partial(wait_in, na, BH - na, 1)]
            done = 0
            for k in range(2, len(segs)):
                wide_lo = segs[k][1][0]
                if wide_lo in OUT_ITERS:
                    hi = NPRE + wide_lo * HB
                    acts[k].append(lambda lo=done, n=hi - done: out_copy(lo, n).start())
                    done = hi

            def narrow(h, carry):
                run_heads([h])
                return carry

            def wide(i, carry):
                h0 = NPRE + i * HB
                run_heads([h0 + u for u in range(HB)])
                return carry

            def bound(i, vals):
                return sum(jnp.where(i == k, v, 0) for k, v in enumerate(vals) if v)

            def segment(i, carry):
                for k, fns in enumerate(acts):
                    if fns:
                        @pl.when(i == k)
                        def _(fns=fns):
                            for f in fns:
                                f()
                lo1 = bound(i, [s[0][0] for s in segs]); hi1 = bound(i, [s[0][1] for s in segs])
                lo4 = bound(i, [s[1][0] for s in segs]); hi4 = bound(i, [s[1][1] for s in segs])
                lax.fori_loop(lo1, hi1, narrow, 0)
                lax.fori_loop(lo4, hi4, wide, 0)
                return carry

            lax.fori_loop(0, len(segs), segment, 0)
            out_copy(done, BH - done).start()
            out_copy(0, BH).wait()

        def general_path():
            wait_in(1, 1, 1)
            GK = 512

            def head(h, carry):
                start_in(h, 1, 0)
                wait_in(h, 1, 0)
                for c in range(NC):
                    prep_kv(h, c)
                th = t_ref[h % H]

                def qtile(j, carry2):
                    q0 = pl.multiple_of(j * BQ, BQ)
                    qq = normalise(q_v[h, :, pl.ds(q0, BQ)], 1.0).astype(bf16)
                    w = jnp.concatenate([qq, jnp.zeros((128 - D, BQ), bf16)], axis=0)

                    def kblock(kb, st):
                        m, l, acc = st
                        k0 = pl.multiple_of(kb * (GK // 2), GK // 2)
                        kk = pltpu.bitcast(kn[pl.ds(k0, GK // 2), :], bf16)
                        s = jnp.dot(kk, w, preferred_element_type=f32) * th
                        m_new = jnp.maximum(m, jnp.max(s, axis=0, keepdims=True))
                        alpha = jnp.exp(m - m_new)
                        p = jnp.exp(s - m_new)
                        l = alpha * l + jnp.sum(p, axis=0, keepdims=True)
                        v0 = pl.multiple_of(kb * GK, GK)
                        vv = pltpu.bitcast(vn[:, pl.ds(v0, GK)], bf16)
                        acc = alpha * acc + jnp.dot(vv, p.astype(bf16), preferred_element_type=f32)
                        return m_new, l, acc

                    init = (jnp.full((1, BQ), -jnp.inf, f32), jnp.zeros((1, BQ), f32), jnp.zeros((D, BQ), f32))
                    m, l, acc = lax.fori_loop(0, S // GK, kblock, init)
                    o_v[h, :, pl.ds(q0, BQ)] = (acc / l).astype(bf16)
                    return carry2

                lax.fori_loop(0, NP, qtile, 0)
                out_copy(h, 1).start()
                out_copy(h, 1).wait()
                return carry

            lax.fori_loop(0, BH, head, 0)

        start_in(0, 1, 0)
        start_in(1, 1, 1)
        safe = functools.reduce(jnp.logical_and, [jnp.abs(t_ref[i]) <= T_SAFE for i in range(H)])
        wait_in(0, 1, 0)
        pl.when(safe)(fast_path)
        pl.when(jnp.logical_not(safe))(general_path)

    slab = pltpu.VMEM((BH, D, S), bf16)
    scratch = [slab, slab, slab, slab,
               pltpu.VMEM((S // 2, 128), u32),
               pltpu.VMEM((D // 2 + 8, S), u32),
               pltpu.VMEM((D // 2, S), u32),
               pltpu.SemaphoreType.DMA((2,)), pltpu.SemaphoreType.DMA((1,))]
    return kernel, scratch


def _impl(q, k, v, t, **cfg):
    B, H, S, D = q.shape
    BH = B * H
    kernel, scratch = make_kernel(B, H, S, D, **cfg)
    to_t = lambda x: jnp.swapaxes(x, -1, -2).reshape(BH, D, S)
    anyspec = pl.BlockSpec(memory_space=pl.ANY)
    out = pl.pallas_call(
        kernel,
        in_specs=[pl.BlockSpec(memory_space=pltpu.SMEM), anyspec, anyspec, anyspec],
        out_specs=anyspec,
        out_shape=jax.ShapeDtypeStruct((BH, D, S), q.dtype),
        scratch_shapes=scratch,
        compiler_params=pltpu.CompilerParams(vmem_limit_bytes=48 * 1024 * 1024),
    )(t.astype(f32), to_t(q), to_t(k), to_t(v))
    return jnp.swapaxes(out.reshape(B, H, D, S), -1, -2)


@jax.jit
def pallas_standalone__qk_norm__prompt_kernel(q: jax.Array, k: jax.Array, v: jax.Array, t: jax.Array):
    return _impl(q, k, v, t)
```

```python
import functools

import jax
import jax.numpy as jnp
from jax import lax
from jax.experimental import pallas as pl
from jax.experimental.pallas import tpu as pltpu

f32 = jnp.float32
bf16 = jnp.bfloat16
u32 = jnp.uint32

EPS = 1e-6
LOG2E = 1.4426950408889634
T_SAFE = 16.0

CH = 128
BQ = 512
LAG = 2
TAIL = 6
KLEAD = 2
HB = 5
NPRE = 3
NPOST = 1
OUT_ITERS = (1, 6)


def _make_kernel(B, H, S, D):
    BH = B * H
    NC = S // CH
    NP = S // BQ
    LEAD = max(KLEAD * CH, BQ)
    NWIDE = (BH - NPRE - NPOST) // HB
    NA = NPRE + HB + 1
    assert D == 32 and S % BQ == 0 and BH & (BH - 1) == 0
    assert (BH - NPRE - NPOST) % HB == 0 and NPRE >= 2 and NWIDE > max(OUT_ITERS)
    assert KLEAD - 1 < NC - TAIL - LAG and LAG + KLEAD + 1 <= NC

    def kernel(t_hbm, q_hbm, k_hbm, v_hbm, o_hbm,
               t_ref, q_v, k_v, v_v, o_v, kn, qn, vn, in_sem, out_sem):

        def in_copies(lo, n, si, c0=0, nc=S):
            return [pltpu.make_async_copy(src.at[pl.ds(lo, n), :, pl.ds(c0, nc)],
                                          dst.at[pl.ds(lo, n), :, pl.ds(c0, nc)], in_sem.at[si])
                    for src, dst in ((k_hbm, k_v), (q_hbm, q_v), (v_hbm, v_v))]

        def start_in(*a):
            for cp in in_copies(*a):
                cp.start()

        def wait_in(*a):
            for cp in in_copies(*a):
                cp.wait()

        def out_copy(lo, n):
            return pltpu.make_async_copy(o_v.at[pl.ds(lo, n)], o_hbm.at[pl.ds(lo, n)], out_sem.at[0])

        def normalise(x_bf16, scale):
            x = x_bf16.astype(f32)
            ss = jnp.sum(x * x, axis=0, keepdims=True)
            return x * (scale / (jnp.sqrt(ss) + EPS))

        def prep_kv(h, c):
            cols = slice(c * CH, (c + 1) * CH)
            kk = normalise(k_v[h, :, cols], 1.0)
            row = lax.broadcasted_iota(jnp.int32, (8, CH), 0)
            one = jnp.where(row == 0, 1.0, 0.0).astype(f32)
            y = jnp.concatenate([kk, one, jnp.zeros((128 - D - 8, CH), f32)], axis=0)
            kn[c * (CH // 2):(c + 1) * (CH // 2), :] = pltpu.bitcast(y.T.astype(bf16), u32)
            vn[:, cols] = pltpu.bitcast(v_v[h, :, cols], u32)

        def prep_q(h, j):
            cols = slice(j * BQ, (j + 1) * BQ)
            c = t_ref[h % H].astype(f32) * LOG2E
            qq = normalise(q_v[h, :, cols], c)
            qn[0:D // 2, cols] = pltpu.bitcast(qq.astype(bf16), u32)
            row = lax.broadcasted_iota(jnp.int32, (16, BQ), 0)
            shift = jnp.where(row == 0, -jnp.abs(c), 0.0).astype(f32)
            qn[D // 2:D // 2 + 8, cols] = pltpu.bitcast(shift.astype(bf16), u32)

        def qk_exp(j, c):
            w = jnp.concatenate([qn[:, j * BQ:(j + 1) * BQ],
                                 jnp.zeros((64 - D // 2 - 8, BQ), u32)], axis=0)
            kk = pltpu.bitcast(kn[c * (CH // 2):(c + 1) * (CH // 2), :], bf16)
            s = jnp.dot(kk, pltpu.bitcast(w, bf16), preferred_element_type=f32)
            p = jnp.exp2(s)
            return jnp.sum(p.reshape(CH // 8, 8, BQ), axis=0), p.astype(bf16)

        def pv(c, p):
            vv = pltpu.bitcast(vn[:, c * CH:(c + 1) * CH], bf16)
            return jnp.dot(vv, p, preferred_element_type=f32)

        def finish(h, j, l, acc):
            lt = jnp.sum(l, axis=0, keepdims=True)
            o_v[h, :, j * BQ:(j + 1) * BQ] = (acc * (1.0 / lt)).astype(bf16)

        def run_heads(heads):
            blocks = []
            for h in heads:
                hn = jnp.minimum(h + 1, BH - 1)
                for j in range(NP):
                    pre = [[] for _ in range(NC)]
                    if j == 0:
                        for c in range(KLEAD, NC):
                            pre[c - KLEAD].append(functools.partial(prep_kv, h, c))
                    if j + 1 < NP:
                        pre[NC // 2].append(functools.partial(prep_q, h, j + 1))
                    else:
                        pre[NC // 2].append(functools.partial(prep_q, hn, 0))
                        for c in range(KLEAD):
                            pre[NC - 1].append(functools.partial(prep_kv, hn, c))
                    blocks += [(h, j, c, pre[c]) for c in range(NC)]
            n = len(blocks)
            probs, sums, accs = {}, {}, {}
            issued = 0

            def issue_pv(upto):
                nonlocal issued
                while issued < upto:
                    h, j, c, _ = blocks[issued]
                    key = issued // NC
                    r = pv(c, probs.pop(issued))
                    accs[key] = r if c == 0 else accs[key] + r
                    if c == NC - 1:
                        finish(h, j, sums.pop(key), accs.pop(key))
                    issued += 1

            for i, (h, j, c, pre) in enumerate(blocks):
                for f in pre:
                    f()
                ps, probs[i] = qk_exp(j, c)
                sums[i // NC] = ps if c == 0 else sums[i // NC] + ps
                issue_pv(min(i - LAG + 1, n - TAIL - LAG + 1))
            issue_pv(n)

        def fast_path():
            for c in range(KLEAD):
                prep_kv(0, c)
            prep_q(0, 0)

            cuts = [1, *(x for x in OUT_ITERS if x > 1), NWIDE]
            segs = [((0, 1), (0, 0)), ((1, NPRE), (0, 1))]
            segs += [((0, 0), (a, b)) for a, b in zip(cuts[:-1], cuts[1:])]
            segs += [((BH - NPOST, BH), (0, 0))]
            acts = [[] for _ in segs]
            P = functools.partial
            acts[0] += [P(wait_in, 0, 1, 1, LEAD, S - LEAD), P(wait_in, 1, 1, 1, 0, LEAD),
                        P(start_in, 1, 1, 0, LEAD, S - LEAD), P(start_in, 2, NA - 2, 1)]
            acts[1] += [P(wait_in, 1, 1, 0, LEAD, S - LEAD), P(wait_in, 2, NA - 2, 1),
                        P(start_in, NA, BH - NA, 1)]
            acts[2] += [P(wait_in, NA, BH - NA, 1)]
            copied = 0
            for i in range(2, len(segs)):
                single, wide = segs[i]
                done = single[0] if single[1] > single[0] else NPRE + wide[0] * HB
                if single[1] > single[0] or wide[0] in OUT_ITERS:
                    acts[i].append(lambda lo=copied, n=done - copied: out_copy(lo, n).start())
                    copied = done

            def pick(i, vals):
                return sum(jnp.where(i == s, v, 0) for s, v in enumerate(vals) if v)

            def segment(i, carry):
                for s, fns in enumerate(acts):
                    if fns:
                        @pl.when(i == s)
                        def _(fns=fns):
                            for f in fns:
                                f()

                @pl.loop(pick(i, [s[0][0] for s in segs]), pick(i, [s[0][1] for s in segs]))
                def _(h):
                    run_heads([h])

                @pl.loop(pick(i, [s[1][0] for s in segs]), pick(i, [s[1][1] for s in segs]))
                def _(w):
                    run_heads([NPRE + w * HB + u for u in range(HB)])

                return carry

            lax.fori_loop(0, len(segs), segment, 0)
            out_copy(copied, BH - copied).start()
            out_copy(0, BH).wait()

        def general_path():
            wait_in(0, 1, 1, LEAD, S - LEAD)
            wait_in(1, 1, 1, 0, LEAD)
            GK = 512

            @pl.loop(0, BH)
            def _(h):
                start_in(h, 1, 0)
                wait_in(h, 1, 0)
                for c in range(NC):
                    prep_kv(h, c)
                th = t_ref[h % H].astype(f32)

                @pl.loop(0, NP)
                def _(j):
                    q0 = pl.multiple_of(j * BQ, BQ)
                    qq = normalise(q_v[h, :, pl.ds(q0, BQ)], 1.0).astype(bf16)
                    w = jnp.concatenate([qq, jnp.zeros((128 - D, BQ), bf16)], axis=0)

                    def kblock(kb, state):
                        m, l, acc = state
                        k0 = pl.multiple_of(kb * (GK // 2), GK // 2)
                        kk = pltpu.bitcast(kn[pl.ds(k0, GK // 2), :], bf16)
                        s = jnp.dot(kk, w, preferred_element_type=f32) * th
                        m_new = jnp.maximum(m, jnp.max(s, axis=0, keepdims=True))
                        alpha = jnp.exp(m - m_new)
                        p = jnp.exp(s - m_new)
                        l = alpha * l + jnp.sum(p, axis=0, keepdims=True)
                        v0 = pl.multiple_of(kb * GK, GK)
                        vv = pltpu.bitcast(vn[:, pl.ds(v0, GK)], bf16)
                        acc = alpha * acc + jnp.dot(vv, p.astype(bf16), preferred_element_type=f32)
                        return m_new, l, acc

                    init = (jnp.full((1, BQ), -jnp.inf, f32), jnp.zeros((1, BQ), f32),
                            jnp.zeros((D, BQ), f32))
                    _, l, acc = lax.fori_loop(0, S // GK, kblock, init)
                    o_v[h, :, pl.ds(q0, BQ)] = (acc / l).astype(bf16)

                out_copy(h, 1).start()
                out_copy(h, 1).wait()

        t_copy = pltpu.make_async_copy(t_hbm, t_ref, out_sem.at[0])
        t_copy.start()
        start_in(0, 1, 0, 0, LEAD)
        start_in(0, 1, 1, LEAD, S - LEAD)
        start_in(1, 1, 1, 0, LEAD)
        t_copy.wait()
        safe = functools.reduce(
            jnp.logical_and, [jnp.abs(t_ref[i].astype(f32)) <= T_SAFE for i in range(H)])
        wait_in(0, 1, 0, 0, LEAD)
        pl.when(safe)(fast_path)
        pl.when(jnp.logical_not(safe))(general_path)

    slab = pltpu.VMEM((BH, D, S), bf16)
    scratch = [pltpu.SMEM((H,), bf16),
               slab, slab, slab, slab,
               pltpu.VMEM((S // 2, 128), u32),
               pltpu.VMEM((D // 2 + 8, S), u32),
               pltpu.VMEM((D // 2, S), u32),
               pltpu.SemaphoreType.DMA((2,)),
               pltpu.SemaphoreType.DMA((1,))]
    return kernel, scratch


def _impl(q, k, v, t):
    B, H, S, D = q.shape
    kernel, scratch = _make_kernel(B, H, S, D)
    transposed = lambda x: jnp.swapaxes(x, -1, -2).reshape(B * H, D, S)
    hbm = pl.BlockSpec(memory_space=pl.ANY)
    out = pl.pallas_call(
        kernel,
        in_specs=[hbm] * 4,
        out_specs=hbm,
        out_shape=jax.ShapeDtypeStruct((B * H, D, S), q.dtype),
        scratch_shapes=scratch,
        compiler_params=pltpu.CompilerParams(vmem_limit_bytes=48 * 1024 * 1024),
    )(t, transposed(q), transposed(k), transposed(v))
    return jnp.swapaxes(out.reshape(B, H, D, S), -1, -2)


@jax.jit
def pallas_standalone__qk_norm__prompt_kernel(
    q: jax.Array,
    k: jax.Array,
    v: jax.Array,
    t: jax.Array,
):
    return _impl(q, k, v, t)
```
